```python
import os as _os
_os.environ.setdefault("JAX_PLATFORMS", "cpu")
import jax
import jax.numpy as jnp

def _softmax(x, axis=-1):
    return jax.nn.softmax(x, axis=axis)
def _gelu(x):
    return jax.nn.gelu(x, approximate=True)
def _silu(x):
    return jax.nn.silu(x)
def _sigmoid(x):
    return jax.nn.sigmoid(x)
def _layernorm(x, axis=-1, eps=1e-5):
    m = jnp.mean(x, axis=axis, keepdims=True)
    v = jnp.var(x, axis=axis, keepdims=True)
    return (x - m) / jnp.sqrt(v + eps)
def _scatter_add(tgt, idx, src, axis=0):
    return tgt.at[idx].add(src)
def _segment_sum(src, seg, n):
    return jax.ops.segment_sum(src, seg, n)
class _Rng:
    def __init__(self, key):
        self._k = key
    def _next(self):
        self._k, sub = jax.random.split(self._k)
        return sub
    def normal(self, shape):
        return jax.random.normal(self._next(), shape, dtype=jnp.bfloat16)
    def randint(self, lo, hi, shape):
        return jax.random.randint(self._next(), shape, lo, hi, dtype=jnp.int32)
    def uniform(self, shape, lo=0.0, hi=1.0):
        return jax.random.uniform(self._next(), shape, jnp.bfloat16, lo, hi)
    def permutation(self, n):
        return jax.random.permutation(self._next(), n)


kernel_name = 'standalone__gqa_softmax__near_ridge'

def setup_inputs():
    _rng = _Rng(jax.random.key(int.from_bytes(__import__("os").urandom(4), "little")))
    _w = (lambda a: (lambda t: t.astype(jnp.bfloat16) if jnp.issubdtype(t.dtype, jnp.floating) else t)(jnp.asarray(a)))
    B, Hq, Hkv, Sq, Sk, D = 8, 16, 8, 160, 2048, 256
    return {
        "q": _w((lambda *s: _rng.normal(s) * 0.05)(B, Hq, Sq, D)),
        "k": _w((lambda *s: _rng.normal(s) * 3.2)(B, Hkv, Sk, D)),
        "v": _w((lambda *s: _rng.normal(s) * 0.05)(B, Hkv, Sk, D)),
    }

def reference(q, k, v):
    B, Hq, Sq, D = q.shape
    Hkv = k.shape[1]
    rep = Hq // Hkv
    k = jnp.repeat(k, rep, axis=1)
    v = jnp.repeat(v, rep, axis=1)
    scale = D ** -0.5
    scores = jnp.einsum("bhqd,bhkd->bhqk", q, k) * scale
    p = _softmax(scores, axis=-1)
    return jnp.einsum("bhqk,bhkd->bhqd", p, v)
```

```python
import jax
import jax.numpy as jnp
from jax import lax
import jax.experimental.pallas as pl
import jax.experimental.pallas.tpu as pltpu

_CHUNK = 512


def _kernel(q_ref, k_ref, v_ref, o_ref):
    M, D = q_ref.shape[-2:]
    Sk = k_ref.shape[-2]
    scale = D ** -0.5
    q = q_ref[0] * jnp.asarray(scale, q_ref.dtype)
    m = jnp.full((M, 1), -jnp.inf, jnp.float32)
    l = jnp.zeros((M, 1), jnp.float32)
    acc = jnp.zeros((M, D), jnp.float32)
    for j in range(Sk // _CHUNK):
        k = k_ref[0, j * _CHUNK:(j + 1) * _CHUNK, :]
        v = v_ref[0, j * _CHUNK:(j + 1) * _CHUNK, :]
        s = lax.dot_general(q, k, (((1,), (1,)), ((), ())),
                            preferred_element_type=jnp.float32)
        m_new = jnp.maximum(m, s.max(-1, keepdims=True))
        p = jnp.exp(s - m_new)
        alpha = jnp.exp(m - m_new)
        l = alpha * l + p.sum(-1, keepdims=True)
        acc = alpha * acc + jnp.dot(p.astype(v.dtype), v,
                                    preferred_element_type=jnp.float32)
        m = m_new
    o_ref[0] = (acc / l).astype(o_ref.dtype)


@jax.jit
def pallas_standalone__gqa_softmax__near_ridge_kernel(
    q: jax.Array,
    k: jax.Array,
    v: jax.Array,
):
    B, Hq, Sq, D = q.shape
    Hkv, Sk = k.shape[1], k.shape[2]
    rep = Hq // Hkv
    M = rep * Sq
    G = B * Hkv
    q3 = q.reshape(G, M, D)
    k3 = k.reshape(G, Sk, D)
    v3 = v.reshape(G, Sk, D)
    out = pl.pallas_call(
        _kernel,
        grid=(G,),
        in_specs=[pl.BlockSpec((1, M, D), lambda i: (i, 0, 0)),
                  pl.BlockSpec((1, Sk, D), lambda i: (i, 0, 0)),
                  pl.BlockSpec((1, Sk, D), lambda i: (i, 0, 0))],
        out_specs=pl.BlockSpec((1, M, D), lambda i: (i, 0, 0)),
        out_shape=jax.ShapeDtypeStruct((G, M, D), q.dtype),
        compiler_params=pltpu.CompilerParams(
            dimension_semantics=("parallel",),
            vmem_limit_bytes=64 * 1024 * 1024),
    )(q3, k3, v3)
    return out.reshape(B, Hq, Sq, D)
```

```python
import functools
import math

import jax
import jax.numpy as jnp
from jax import lax
import jax.experimental.pallas as pl
import jax.experimental.pallas.tpu as pltpu

_LOG2E = math.log2(math.e)


def _ilog2(x):
    r = int(x).bit_length() - 1
    assert (1 << r) == x, x
    return r


def _lane_sum(p):
    n = p.shape[1] // 128
    parts = [p[:, t * 128:(t + 1) * 128] for t in range(n)]
    while len(parts) > 1:
        nxt = [parts[i] + parts[i + 1] for i in range(0, len(parts) - 1, 2)]
        if len(parts) % 2:
            nxt.append(parts[-1])
        parts = nxt
    return parts[0]


def _head_body(q_at, k_at, v_at, D, n, pre, hook):
    c = (D ** -0.5) * _LOG2E
    m = l = acc = None
    for j in range(n):
        pre(j)
        k = k_at(j)
        q = q_at()
        s = lax.dot_general(q, k, (((1,), (1,)), ((), ())),
                            preferred_element_type=jnp.float32)
        hook(j)
        mc = s.max(-1, keepdims=True)
        m_new = mc if j == 0 else jnp.maximum(m, mc)
        p = jnp.exp2((s - m_new) * c)
        part = _lane_sum(p)
        v = v_at(j)
        pv = jnp.dot(p.astype(v.dtype), v, preferred_element_type=jnp.float32)
        if j == 0:
            l = part
            acc = pv
            alpha = None
        else:
            alpha = jnp.exp2((m - m_new) * c)
            l = alpha * l + part
        if j == n - 1:
            ls = l.sum(-1, keepdims=True)
            r = pl.reciprocal(ls, approx=True)
            inv = r * (2.0 - ls * r)
            if alpha is None:
                return pv * inv
            return acc * (alpha * inv) + pv * inv
        if j > 0:
            acc = alpha * acc + pv
        m = m_new


def _make_kernel(chunk, peel, peel_extra, phases, NB, top_issue):
    def kernel(q_hbm, k_hbm, v_hbm, o_hbm, big, sem_in, sem_peel, sem_out):
        G, M, D = q_hbm.shape
        Sk = k_hbm.shape[1]
        nc = Sk // chunk
        qc = M // nc
        total = G * nc
        SR = 2 * Sk + M
        OB = NB * SR
        npc = sum(peel)
        assert npc % nc == 0
        nph = npc // nc
        assert nph + sum(p[0] * p[1] for p in phases) == G
        lnc = _ilog2(nc)
        _ilog2(NB)
        n_def = nph + sum(p[0] * p[1] for p in phases if p[4])
        region_of = []
        region_start = {}
        for r, sz in enumerate(peel):
            region_start[len(region_of)] = r
            region_of += [r] * sz

        def rows(base, off, size):
            if isinstance(base + off, int):
                return pl.ds(base + off, size)
            return pl.ds(pl.multiple_of(base + off, 16), size)

        def issue_peel(c):
            g, j = divmod(c, nc)
            base = (g % NB) * SR
            sem = sem_peel.at[region_of[c]]
            if j == 0:
                pltpu.make_async_copy(
                    q_hbm.at[g], big.at[rows(base, 2 * Sk, M)], sem).start()
            pltpu.make_async_copy(
                k_hbm.at[g, pl.ds(j * chunk, chunk)],
                big.at[rows(base, j * chunk, chunk)], sem).start()
            pltpu.make_async_copy(
                v_hbm.at[g, pl.ds(j * chunk, chunk)],
                big.at[rows(base, Sk + j * chunk, chunk)], sem).start()

        def wait_peel(c0, r):
            nrows = sum(2 * chunk + (M if c % nc == 0 else 0)
                        for c in range(c0, c0 + peel[r]))
            ref = big.at[pl.ds(0, nrows)]
            pltpu.make_async_copy(ref, ref, sem_peel.at[r]).wait()

        def issue(c, cond=None):
            if isinstance(c, int):
                if c < npc:
                    return issue_peel(c)
                if c >= total:
                    return
                c = jnp.int32(c)
            ok = c < total
            if cond is not None:
                ok = jnp.logical_and(ok, cond)

            @pl.when(ok)
            def _():
                g = lax.shift_right_logical(c, lnc)
                j = c & (nc - 1)
                slot = g & (NB - 1)
                base = slot * SR
                ko = pl.multiple_of(j * chunk, chunk)
                qo = pl.multiple_of(j * qc, qc)
                pltpu.make_async_copy(
                    k_hbm.at[g, pl.ds(ko, chunk)],
                    big.at[rows(base, ko, chunk)], sem_in.at[slot]).start()
                pltpu.make_async_copy(
                    v_hbm.at[g, pl.ds(ko, chunk)],
                    big.at[rows(base, Sk + ko, chunk)], sem_in.at[slot]).start()
                pltpu.make_async_copy(
                    q_hbm.at[g, pl.ds(qo, qc)],
                    big.at[rows(base, 2 * Sk + qo, qc)], sem_in.at[slot]).start()

        def wait_in(slot):
            r = big.at[rows(slot * SR, 0, SR)]
            pltpu.make_async_copy(r, r, sem_in.at[slot]).wait()

        def out_start(g):
            pltpu.make_async_copy(
                big.at[rows(OB, g * M, M)], o_hbm.at[g], sem_out).start()

        def run_head(base, pre, hook):
            return _head_body(
                lambda: big[rows(base, 2 * Sk, M), :],
                lambda j: big[rows(base, j * chunk, chunk), :],
                lambda j: big[rows(base, Sk + j * chunk, chunk), :],
                D, nc, pre, hook)

        fr = [peel[0]]
        for c in range(peel[0]):
            issue(c)

        def adv(k):
            for _ in range(k):
                issue(fr[0])
                fr[0] += 1

        pend = []

        def flush_peel():
            while pend:
                gg, o = pend.pop(0)
                big[rows(OB, gg * M, M), :] = o.astype(big.dtype)

        for g in range(nph):
            def pre(j, g=g):
                c = g * nc + j
                if c in region_start:
                    r = region_start[c]
                    assert fr[0] >= c + peel[r], ("peel deadlock", c, fr[0])
                    wait_peel(c, r)
                    if r == 0:
                        adv(top_issue)

            def hook(j, g=g):
                c = g * nc + j
                if j == 0:
                    flush_peel()
                adv(1 + sum(1 for e in peel_extra if e == c))

            pend.append((g, run_head((g % NB) * SR, pre, hook)))
        flush_peel()
        f0 = fr[0]
        assert (min(f0, total) - 1) // nc <= NB - 1

        _f, _a = f0, nph
        for (_n, _N, _ev, _cnt, _d, _c) in phases:
            for _i in range(_N):
                assert min(_f, total) >= nc * (_a + _n), ("deadlock", _a, _f)
                _f += _n * nc + (_cnt if _i % _ev == 0 else 0)
                assert (min(_f, total) - 1) // nc <= _a + NB - 1, ("slot reuse", _a, _f)
                _a += _n

        front_static, a_static, of_static = f0, nph, 0
        for (n, N, every, cnt, defer, catch) in phases:
            def step(i, front, n=n, every=every, cnt=cnt, a0=a_static,
                     defer=defer, catch=catch, of0=of_static):
                a = a0 + i * n
                for h in range(n):
                    wait_in((a + h) & (NB - 1))
                do = None
                if cnt > 0 and every > 1:
                    do = (i % every) == 0
                    nextra = jnp.where(do, cnt, 0)
                else:
                    nextra = cnt
                pending = []

                def flush():
                    while pending:
                        g, o = pending.pop(0)
                        big[rows(OB, g * M, M), :] = o.astype(big.dtype)
                        if not defer:
                            out_start(g)

                def hook(h, j):
                    idx = h * nc + j
                    if j == 0:
                        flush()
                    if idx == 0:
                        for e in range(cnt):
                            issue(front + e, do)
                    issue(front + idx + nextra)
                    if catch and idx % 2 == 1 and idx // 2 < catch:
                        og = of0 + i * catch + idx // 2

                        @pl.when(og < n_def)
                        def _():
                            out_start(og)

                for h in range(n):
                    base = ((a + h) & (NB - 1)) * SR
                    o = run_head(base, lambda j: None, functools.partial(hook, h))
                    pending.append((a + h, o))
                flush()
                return front + n * nc + nextra

            lax.fori_loop(0, N, step, jnp.int32(front_static))
            front_static += N * n * nc + (-(-N // every)) * cnt
            a_static += n * N
            of_static = min(n_def, of_static + N * catch)
        assert front_static >= total
        for g in range(of_static, n_def):
            out_start(g)
        o_all = big.at[pl.ds(OB, G * M)]
        pltpu.make_async_copy(o_all, o_all, sem_out).wait()

    return kernel


@jax.jit
def pallas_standalone__gqa_softmax__near_ridge_kernel(
    q: jax.Array,
    k: jax.Array,
    v: jax.Array,
):
    B, Hq, Sq, D = q.shape
    Hkv, Sk = k.shape[1], k.shape[2]
    rep = Hq // Hkv
    M = rep * Sq
    G = B * Hkv
    q3 = q.reshape(G, M, D)
    k3 = k.reshape(G, Sk, D)
    v3 = v.reshape(G, Sk, D)

    chunk, NB = 512, 16
    peel = (2, 2, 2, 3, 3)
    peel_extra = (3, 7, 9)
    phases = ((1, 7, 1, 1, True, 0), (2, 7, 1, 1, True, 0), (4, 10, 1, 1, False, 3))
    assert G == 64 and Sk == 2048 and M % 64 == 0

    out = pl.pallas_call(
        _make_kernel(chunk, peel, peel_extra, phases, NB, top_issue=1),
        in_specs=[pl.BlockSpec(memory_space=pl.ANY)] * 3,
        out_specs=pl.BlockSpec(memory_space=pl.ANY),
        out_shape=jax.ShapeDtypeStruct((G, M, D), q.dtype),
        scratch_shapes=[
            pltpu.VMEM((NB * (2 * Sk + M) + G * M, D), k.dtype),
            pltpu.SemaphoreType.DMA((NB,)),
            pltpu.SemaphoreType.DMA((len(peel),)),
            pltpu.SemaphoreType.DMA(()),
        ],
        compiler_params=pltpu.CompilerParams(
            vmem_limit_bytes=100 * 1024 * 1024,
            disable_bounds_checks=True),
    )(q3, k3, v3)
    return out.reshape(B, Hq, Sq, D)
```

```python
import functools
import math

import jax
import jax.numpy as jnp
from jax import lax
import jax.experimental.pallas as pl
import jax.experimental.pallas.tpu as pltpu

_LOG2E = math.log2(math.e)
_OSPLIT = 4


def _ilog2(x):
    r = int(x).bit_length() - 1
    assert (1 << r) == x, x
    return r


def _lane_sum(p):
    n = p.shape[1] // 128
    parts = [p[:, t * 128:(t + 1) * 128] for t in range(n)]
    while len(parts) > 1:
        nxt = [parts[i] + parts[i + 1] for i in range(0, len(parts) - 1, 2)]
        if len(parts) % 2:
            nxt.append(parts[-1])
        parts = nxt
    return parts[0]


def _head_body(q_at, k_at, v_at, D, n, pre, hook):
    c = (D ** -0.5) * _LOG2E
    m = l = acc = None
    for j in range(n):
        pre(j)
        k = k_at(j)
        q = q_at()
        s = lax.dot_general(q, k, (((1,), (1,)), ((), ())),
                            preferred_element_type=jnp.float32)
        hook(j)
        mc = s.max(-1, keepdims=True)
        m_new = mc if j == 0 else jnp.maximum(m, mc)
        p = jnp.exp2((s - m_new) * c)
        part = _lane_sum(p)
        v = v_at(j)
        pv = jnp.dot(p.astype(v.dtype), v, preferred_element_type=jnp.float32)
        if j == 0:
            l = part
            acc = pv
            alpha = None
        else:
            alpha = jnp.exp2((m - m_new) * c)
            l = alpha * l + part
        if j == n - 1:
            ls = l.sum(-1, keepdims=True)
            r = pl.reciprocal(ls, approx=True)
            inv = r * (2.0 - ls * r)
            if alpha is None:
                return pv * inv
            return acc * (alpha * inv) + pv * inv
        if j > 0:
            acc = alpha * acc + pv
        m = m_new


def _make_kernel(chunk, peel, peel_extra, phases, NB, top_issue):
    def kernel(q_hbm, k_hbm, v_hbm, o_hbm, big, sem_in, sem_peel, sem_out):
        G, M, D = q_hbm.shape
        Sk = k_hbm.shape[1]
        nc = Sk // chunk
        qc = M // nc
        total = G * nc
        SR = 2 * Sk + M
        OB = NB * SR
        npc = sum(peel)
        assert npc % nc == 0
        nph = npc // nc
        assert nph + sum(p[0] * p[1] for p in phases) == G
        lnc = _ilog2(nc)
        _ilog2(NB)
        n_def = nph + sum(p[0] * p[1] for p in phases if p[4])
        region_of = []
        region_start = {}
        for r, sz in enumerate(peel):
            region_start[len(region_of)] = r
            region_of += [r] * sz

        def rows(base, off, size):
            if isinstance(base + off, int):
                return pl.ds(base + off, size)
            return pl.ds(pl.multiple_of(base + off, 16), size)

        def issue_peel(c):
            g, j = divmod(c, nc)
            base = (g % NB) * SR
            sem = sem_peel.at[region_of[c]]
            if j == 0:
                pltpu.make_async_copy(
                    q_hbm.at[g], big.at[rows(base, 2 * Sk, M)], sem).start()
            pltpu.make_async_copy(
                k_hbm.at[g, pl.ds(j * chunk, chunk)],
                big.at[rows(base, j * chunk, chunk)], sem).start()
            pltpu.make_async_copy(
                v_hbm.at[g, pl.ds(j * chunk, chunk)],
                big.at[rows(base, Sk + j * chunk, chunk)], sem).start()

        def wait_peel(c0, r):
            nrows = sum(2 * chunk + (M if c % nc == 0 else 0)
                        for c in range(c0, c0 + peel[r]))
            ref = big.at[pl.ds(0, nrows)]
            pltpu.make_async_copy(ref, ref, sem_peel.at[r]).wait()

        def issue(c, cond=None):
            if isinstance(c, int):
                if c < npc:
                    return issue_peel(c)
                if c >= total:
                    return
                c = jnp.int32(c)
            ok = c < total
            if cond is not None:
                ok = jnp.logical_and(ok, cond)

            @pl.when(ok)
            def _():
                g = lax.shift_right_logical(c, lnc)
                j = c & (nc - 1)
                slot = g & (NB - 1)
                base = slot * SR
                ko = pl.multiple_of(j * chunk, chunk)
                qo = pl.multiple_of(j * qc, qc)
                pltpu.make_async_copy(
                    k_hbm.at[g, pl.ds(ko, chunk)],
                    big.at[rows(base, ko, chunk)], sem_in.at[slot]).start()
                pltpu.make_async_copy(
                    v_hbm.at[g, pl.ds(ko, chunk)],
                    big.at[rows(base, Sk + ko, chunk)], sem_in.at[slot]).start()
                pltpu.make_async_copy(
                    q_hbm.at[g, pl.ds(qo, qc)],
                    big.at[rows(base, 2 * Sk + qo, qc)], sem_in.at[slot]).start()

        def wait_in(slot):
            r = big.at[rows(slot * SR, 0, SR)]
            pltpu.make_async_copy(r, r, sem_in.at[slot]).wait()

        def out_start(g):
            pltpu.make_async_copy(
                big.at[rows(OB, g * M, M)], o_hbm.at[g], sem_out).start()

        def run_head(base, pre, hook):
            return _head_body(
                lambda: big[rows(base, 2 * Sk, M), :],
                lambda j: big[rows(base, j * chunk, chunk), :],
                lambda j: big[rows(base, Sk + j * chunk, chunk), :],
                D, nc, pre, hook)

        fr = [peel[0]]
        for c in range(peel[0]):
            issue(c)

        def adv(k):
            for _ in range(k):
                issue(fr[0])
                fr[0] += 1

        pend = []

        def flush_peel():
            while pend:
                gg, o = pend.pop(0)
                big[rows(OB, gg * M, M), :] = o.astype(big.dtype)

        for g in range(nph):
            def pre(j, g=g):
                c = g * nc + j
                if c in region_start:
                    r = region_start[c]
                    assert fr[0] >= c + peel[r], ("peel deadlock", c, fr[0])
                    wait_peel(c, r)
                    if r == 0:
                        adv(top_issue)

            def hook(j, g=g):
                c = g * nc + j
                if j == 0:
                    flush_peel()
                adv(1 + sum(1 for e in peel_extra if e == c))

            pend.append((g, run_head((g % NB) * SR, pre, hook)))
        flush_peel()
        f0 = fr[0]
        assert (min(f0, total) - 1) // nc <= NB - 1

        _f, _a = f0, nph
        for (_n, _N, _ev, _cnt, _d, _c) in phases:
            for _i in range(_N):
                assert min(_f, total) >= nc * (_a + _n), ("deadlock", _a, _f)
                _f += _n * nc + (_cnt if _i % _ev == 0 else 0)
                assert (min(_f, total) - 1) // nc <= _a + NB - 1, ("slot reuse", _a, _f)
                _a += _n

        front_static, a_static, of_static = f0, nph, 0
        for (n, N, every, cnt, defer, catch) in phases:
            def step(i, front, n=n, every=every, cnt=cnt, a0=a_static,
                     defer=defer, catch=catch, of0=of_static):
                a = a0 + i * n
                for h in range(n):
                    wait_in((a + h) & (NB - 1))
                do = None
                if cnt > 0 and every > 1:
                    do = (i % every) == 0
                    nextra = jnp.where(do, cnt, 0)
                else:
                    nextra = cnt
                pending = []

                def flush(last=False):
                    while pending:
                        g, o = pending.pop(0)
                        if last and not defer:
                            mb = M // _OSPLIT
                            for t in range(_OSPLIT):
                                r = rows(OB, g * M + t * mb, mb)
                                big[r, :] = o[t * mb:(t + 1) * mb].astype(big.dtype)
                                pltpu.make_async_copy(
                                    big.at[r], o_hbm.at[g, pl.ds(t * mb, mb)],
                                    sem_out).start()
                            continue
                        big[rows(OB, g * M, M), :] = o.astype(big.dtype)
                        if not defer:
                            out_start(g)

                def hook(h, j):
                    idx = h * nc + j
                    if j == 0:
                        flush()
                    if idx == 0:
                        for e in range(cnt):
                            issue(front + e, do)
                    issue(front + idx + nextra)
                    if catch and idx % 2 == 1 and idx // 2 < catch:
                        og = of0 + i * catch + idx // 2

                        @pl.when(og < n_def)
                        def _():
                            out_start(og)

                for h in range(n):
                    base = ((a + h) & (NB - 1)) * SR
                    o = run_head(base, lambda j: None, functools.partial(hook, h))
                    pending.append((a + h, o))
                flush(True)
                return front + n * nc + nextra

            lax.fori_loop(0, N, step, jnp.int32(front_static))
            front_static += N * n * nc + (-(-N // every)) * cnt
            a_static += n * N
            of_static = min(n_def, of_static + N * catch)
        assert front_static >= total
        for g in range(of_static, n_def):
            out_start(g)
        o_all = big.at[pl.ds(OB, G * M)]
        pltpu.make_async_copy(o_all, o_all, sem_out).wait()

    return kernel


@jax.jit
def pallas_standalone__gqa_softmax__near_ridge_kernel(
    q: jax.Array,
    k: jax.Array,
    v: jax.Array,
):
    B, Hq, Sq, D = q.shape
    Hkv, Sk = k.shape[1], k.shape[2]
    rep = Hq // Hkv
    M = rep * Sq
    G = B * Hkv
    q3 = q.reshape(G, M, D)
    k3 = k.reshape(G, Sk, D)
    v3 = v.reshape(G, Sk, D)

    chunk, NB = 512, 16
    peel = (2, 2, 2, 3, 3)
    peel_extra = (2, 5, 8, 10)
    phases = ((1, 7, 1, 1, True, 0), (2, 7, 1, 1, True, 0), (4, 10, 1, 1, False, 3))
    assert G == 64 and Sk == 2048 and M % 64 == 0

    out = pl.pallas_call(
        _make_kernel(chunk, peel, peel_extra, phases, NB, top_issue=1),
        in_specs=[pl.BlockSpec(memory_space=pl.ANY)] * 3,
        out_specs=pl.BlockSpec(memory_space=pl.ANY),
        out_shape=jax.ShapeDtypeStruct((G, M, D), q.dtype),
        scratch_shapes=[
            pltpu.VMEM((NB * (2 * Sk + M) + G * M, D), k.dtype),
            pltpu.SemaphoreType.DMA((NB,)),
            pltpu.SemaphoreType.DMA((len(peel),)),
            pltpu.SemaphoreType.DMA(()),
        ],
        compiler_params=pltpu.CompilerParams(
            vmem_limit_bytes=100 * 1024 * 1024,
            disable_bounds_checks=True),
    )(q3, k3, v3)
    return out.reshape(B, Hq, Sq, D)
```
